```python
import jax
import jax.numpy as jnp

def _softmax(x, axis=-1):
    return jax.nn.softmax(x, axis=axis)

def _gelu(x):
    return jax.nn.gelu(x, approximate=True)

def _silu(x):
    return jax.nn.silu(x)

def _sigmoid(x):
    return jax.nn.sigmoid(x)

def _layernorm(x, axis=-1, eps=1e-05):
    m = jnp.mean(x, axis=axis, keepdims=True)
    v = jnp.var(x, axis=axis, keepdims=True)
    return (x - m) / jnp.sqrt(v + eps)

def _scatter_add(tgt, idx, src, axis=0):
    return tgt.at[idx].add(src)

def _segment_sum(src, seg, n):
    return jax.ops.segment_sum(src, seg, n)

class _Rng:

    def __init__(self, key):
        self._k = key

    def _next(self):
        self._k, sub = jax.random.split(self._k)
        return sub

    def normal(self, shape):
        return jax.random.normal(self._next(), shape, dtype=jnp.bfloat16)

    def randint(self, lo, hi, shape):
        return jax.random.randint(self._next(), shape, lo, hi, dtype=jnp.int32)

    def uniform(self, shape, lo=0.0, hi=1.0):
        return jax.random.uniform(self._next(), shape, jnp.bfloat16, lo, hi)

    def permutation(self, n):
        return jax.random.permutation(self._next(), n)
kernel_name = 'concat_heads__ssm_conv_h3__memory_aug_recurrent_mem_tr__prompt'

def setup_inputs():
    _rng = _Rng(jax.random.key(int.from_bytes(__import__("os").urandom(4), "little")))
    _w = lambda a: (lambda t: t.astype(jnp.bfloat16) if jnp.issubdtype(t.dtype, jnp.floating) else t)(jnp.asarray(a))

    def _A_setup():
        B, S, D = (1, 2048, 1024)
        ks = 4
        return {'q': _w((lambda *s: _rng.normal(s) * 0.05)(B, S, D)), 'k': _w((lambda *s: _rng.normal(s) * 0.05)(B, S, D)), 'v': _w((lambda *s: _rng.normal(s) * 0.05)(B, S, D)), 'shift_k': _w((lambda *s: _rng.normal(s) * 0.05)(D, ks) * 0.5), 'ssm_k': _w((lambda *s: _rng.normal(s) * 0.05)(D, S) * (1.0 / S ** 0.5)), 'ssm_D': _w((lambda *s: _rng.normal(s) * 0.05)(D))}
    _A_in = _A_setup()

    def _B_setup():
        B, S, Dm = (1, 2048, 1024)
        H, Dh = (32, 128)
        M, seg = (8, 32)
        seg = min(seg, S)
        S = S // seg * seg
        return {'x': _w((lambda *s: _rng.normal(s) * 0.05)(B, S, Dm)), 'mem0': _w((lambda *s: _rng.normal(s) * 0.05)(B, M, Dm)), 'Wq': _w((lambda *s: _rng.normal(s) * 0.05)(Dm, H, Dh) * Dm ** (-0.5)), 'Wk': _w((lambda *s: _rng.normal(s) * 0.05)(Dm, H, Dh) * Dm ** (-0.5)), 'Wv': _w((lambda *s: _rng.normal(s) * 0.05)(Dm, H, Dh) * Dm ** (-0.5)), 'Wo': _w((lambda *s: _rng.normal(s) * 0.05)(H, Dh, Dm) * (H * Dh) ** (-0.5)), 'seg_len': seg}
    _B_in = _B_setup()
    return {'A_q': _A_in['q'], 'A_k': _A_in['k'], 'A_v': _A_in['v'], 'A_shift_k': _A_in['shift_k'], 'A_ssm_k': _A_in['ssm_k'], 'A_ssm_D': _A_in['ssm_D'], 'B_x': _B_in['x'], 'B_mem0': _B_in['mem0'], 'B_Wq': _B_in['Wq'], 'B_Wk': _B_in['Wk'], 'B_Wv': _B_in['Wv'], 'B_Wo': _B_in['Wo'], 'B_seg_len': _B_in['seg_len']}

def reference(A_q, A_k, A_v, A_shift_k, A_ssm_k, A_ssm_D, B_x, B_mem0, B_Wq, B_Wk, B_Wv, B_Wo, B_seg_len):

    def _A_ref(q, k, v, shift_k, ssm_k, ssm_D):
        B, S, D = q.shape
        ks = shift_k.shape[-1]
        k_pad = jnp.pad(k, ((0, 0), (ks - 1, 0), (0, 0)))
        k_shift = jnp.zeros_like(k)
        for t in range(ks):
            k_shift = k_shift + k_pad[:, t:t + S, :] * shift_k[:, ks - 1 - t][None, None, :]
        kv = k_shift * v
        L = 2 * S
        kv_pad = jnp.pad(kv, ((0, 0), (0, S), (0, 0)))
        kf_pad = jnp.pad(ssm_k, ((0, 0), (0, S)))
        kv_f = (lambda x, axes=(-2, -1): jnp.fft.rfft2(x.astype(jnp.float32), axes=axes))(kv_pad[:, None, :, :], axes=(1, 2))
        kf_f = (lambda x, axes=(-2, -1): jnp.fft.rfft2(x.astype(jnp.float32), axes=axes))(kf_pad[:, None, :], axes=(1, 2))
        kf_f = (lambda x, *d: x.transpose(*d))(kf_f, 1, 2, 0)
        y_f = kv_f * kf_f[None, :, :, :]
        y = (lambda x, s, axes=(-2, -1): jnp.fft.irfft2(x, s=s, axes=axes).astype(jnp.bfloat16))(y_f, (1, L), axes=(1, 2))[:, 0, :S, :]
        y = y + kv * ssm_D[None, None, :]
        return q * y

    def _B_ref(x, mem0, Wq, Wk, Wv, Wo, seg_len):
        B, S, Dm = x.shape
        H, Dh = (Wq.shape[1], Wq.shape[2])
        M = mem0.shape[1]
        scale = Dh ** (-0.5)
        n_seg = S // seg_len
        L = M + seg_len
        idx = jnp.arange(L)
        mask = (idx[:, None] < M) | (idx[:, None] >= idx[None, :])
        mem = mem0
        outs = []
        for s in range(n_seg):
            xs = x[:, s * seg_len:(s + 1) * seg_len, :].copy()
            h = jnp.concatenate([mem, xs], axis=1)
            q = jnp.einsum('btd,dhe->bhte', h, Wq)
            k = jnp.einsum('btd,dhe->bhte', h, Wk)
            v = jnp.einsum('btd,dhe->bhte', h, Wv)
            scores = jnp.einsum('bhqe,bhke->bhqk', q, k) * scale
            scores = jnp.where(mask[None, None], scores, -1000000000.0)
            p = _softmax(scores, axis=-1)
            o = jnp.einsum('bhqk,bhke->bhqe', p, v)
            o = jnp.einsum('bhte,hed->btd', o, Wo)
            mem = o[:, :M, :].copy()
            outs.append(o[:, M:, :])
        return jnp.concatenate(outs, axis=1)
    a = _A_ref(A_q, A_k, A_v, A_shift_k, A_ssm_k, A_ssm_D)
    b = _B_ref(B_x, B_mem0, B_Wq, B_Wk, B_Wv, B_Wo, B_seg_len)
    return jnp.concatenate([a, b], axis=-1)
```

```python
import functools

import jax
import jax.numpy as jnp
import numpy as np
import jax.experimental.pallas as pl
import jax.experimental.pallas.tpu as pltpu

_TB = 128


def _dft_matrices():
    n = np.arange(_TB)
    k = np.concatenate([np.arange(0, _TB, 2), np.arange(1, _TB, 2)])
    ang = np.pi * (((2 * k[:, None] + 1) * n[None, :]) % (4 * _TB)) / (2 * _TB)
    fwd = np.concatenate([np.cos(ang), -np.sin(ang)], axis=0)
    inv = fwd.T / _TB
    return fwd.astype(jnp.bfloat16), inv.astype(jnp.bfloat16)


def _mm(a, b):
    return jax.lax.dot_general(
        a, b, (((1,), (0,)), ((), ())), preferred_element_type=jnp.float32)


def _mm_t(a, b):
    return jax.lax.dot_general(
        a, b, (((1,), (1,)), ((), ())), preferred_element_type=jnp.float32)


def _kernel(q_hbm, k_hbm, v_hbm, sk_ref, hk_hbm, d_ref, x_hbm, mem_ref,
            wq_hbm, wk_hbm, wv_hbm, wo_hbm, f_ref, g_ref,
            out_hbm,
            wq, wk, wv, wo, stage, h_scr, xs, hs, zprev, kpad, skd,
            q_buf, k_buf, v_buf, hk_buf, x_buf, oa_buf, ob_buf,
            w_sem, wo_sem, in_sem, out_sem,
            *, seg, n_seg, n_grp, cg):
    f32, bf16 = jnp.float32, jnp.bfloat16
    dm, nh, dh = wq_hbm.shape
    n_mem = mem_ref.shape[0]
    n_row = n_mem + seg
    n_tb = n_seg // n_grp
    ks = sk_ref.shape[0]
    da = q_hbm.shape[1]
    zero_slot = n_grp * n_tb
    scale = dh ** (-0.5)

    def in_copies(s, slot):
        a, g = s // n_grp, s % n_grp
        t0 = pl.multiple_of(a * _TB, _TB)
        c0 = pl.multiple_of(g * cg, cg)
        r0 = pl.multiple_of(s * seg, seg)
        blk = (pl.ds(t0, _TB), pl.ds(c0, cg))
        return [
            pltpu.make_async_copy(x_hbm.at[pl.ds(r0, seg), :], x_buf.at[slot], in_sem.at[slot, 0]),
            pltpu.make_async_copy(k_hbm.at[blk], k_buf.at[slot], in_sem.at[slot, 1]),
            pltpu.make_async_copy(v_hbm.at[blk], v_buf.at[slot], in_sem.at[slot, 2]),
            pltpu.make_async_copy(q_hbm.at[blk], q_buf.at[slot], in_sem.at[slot, 3]),
            pltpu.make_async_copy(hk_hbm.at[pl.ds(c0, cg), pl.ds(t0, _TB)], hk_buf.at[slot], in_sem.at[slot, 4]),
        ]

    def out_copies(s, slot):
        a, g = s // n_grp, s % n_grp
        t0 = pl.multiple_of(a * _TB, _TB)
        c0 = pl.multiple_of(g * cg, cg)
        r0 = pl.multiple_of(s * seg, seg)
        return [
            pltpu.make_async_copy(oa_buf.at[slot], out_hbm.at[pl.ds(t0, _TB), pl.ds(c0, cg)], out_sem.at[slot, 0]),
            pltpu.make_async_copy(ob_buf.at[slot], out_hbm.at[pl.ds(r0, seg), pl.ds(da, dm)], out_sem.at[slot, 1]),
        ]

    n_stage, dc = stage.shape[0], stage.shape[1]
    n_chunk = dm // dc
    chunks = [(src, dst, c) for src, dst in ((wq_hbm, wq), (wk_hbm, wk), (wv_hbm, wv))
              for c in range(n_chunk)]

    def w_copy(i):
        src, _, c = chunks[i]
        return pltpu.make_async_copy(
            src.at[pl.ds(c * dc, dc)], stage.at[i % n_stage], w_sem.at[i % n_stage])

    wo_copies = [
        pltpu.make_async_copy(wo_hbm.at[:, pl.ds(n * 128, 128)], wo.at[n], wo_sem.at[n])
        for n in range(dm // 128)]

    for i in range(n_stage):
        w_copy(i).start()

    h_scr[0:n_mem, :] = mem_ref[...].astype(f32)
    xs[zero_slot] = jnp.zeros(xs.shape[1:], f32)
    hs[zero_slot] = jnp.zeros(hs.shape[1:], f32)
    zprev[...] = jnp.zeros(zprev.shape, f32)
    kpad[:, 0:8, :] = jnp.zeros((n_grp, 8, cg), f32)
    for g in range(n_grp):
        cols = slice(g * cg, (g + 1) * cg)
        for j in range(ks):
            skd[g, j] = jnp.broadcast_to(sk_ref[j:j + 1, cols].astype(f32), (8, cg))
        skd[g, ks] = jnp.broadcast_to(d_ref[:, cols].astype(f32), (8, cg))

    for i, (_, dst, c) in enumerate(chunks):
        w_copy(i).wait()

        def relayout(j, carry, dst=dst, c=c, buf=i % n_stage):
            r = pl.multiple_of(j * 16, 16)
            dst[:, pl.ds(c * dc + r, 16), :] = jnp.swapaxes(stage[buf, pl.ds(r, 16)], 0, 1)
            return carry

        jax.lax.fori_loop(0, dc // 16, relayout, 0)
        if i + n_stage < len(chunks):
            w_copy(i + n_stage).start()
        elif i + n_stage == len(chunks):
            for cp in wo_copies:
                cp.start()
            for cp in in_copies(0, 0):
                cp.start()
    for cp in wo_copies:
        cp.wait()

    hg = 4
    n_hg = nh // hg

    def step(s, carry):
        slot = s % 2
        a, g = s // n_grp, s % n_grp
        for cp in in_copies(s, slot):
            cp.wait()

        @pl.when(s + 1 < n_seg)
        def _():
            for cp in in_copies(s + 1, 1 - slot):
                cp.start()

        @pl.when(s >= 2)
        def _():
            for cp in out_copies(s - 2, slot):
                cp.wait()

        st = {}

        def a_forward():
            kf = k_buf[slot].astype(f32)
            kpad[g, 8:8 + _TB, :] = kf
            tile = lambda j: jnp.tile(skd[g, j], (_TB // 8, 1))
            acc = kf * tile(0)
            for j in range(1, ks):
                acc = acc + kpad[g, 8 - j:8 - j + _TB, :] * tile(j)
            kpad[g, 0:8, :] = kf[_TB - 8:, :]
            kv = acc * v_buf[slot].astype(f32)
            st["skip"] = kv * tile(ks)
            xs[g * n_tb + a] = _mm(f_ref[...], kv.astype(bf16))
            hs[g * n_tb + a] = _mm_t(f_ref[...], hk_buf[slot])

        def a_mix(r0, nr):
            re, im = pl.ds(r0, nr), pl.ds(_TB + r0, nr)
            zr = zi = None
            for j in range(n_tb):
                ix = jnp.where(j <= a, g * n_tb + a - j, zero_slot)
                ih = jnp.where(j <= a, g * n_tb + j, zero_slot)
                xr, xi, hr, hi = xs[ix, re, :], xs[ix, im, :], hs[ih, re, :], hs[ih, im, :]
                pr, pi = xr * hr - xi * hi, xr * hi + xi * hr
                zr, zi = (pr, pi) if zr is None else (zr + pr, zi + pi)
            qr, qi = zprev[g, re, :], zprev[g, im, :]
            zprev[g, re, :] = zr
            zprev[g, im, :] = zi
            if r0 < _TB // 2:
                yr, yi = zr - qi, zi + qr
            else:
                yr, yi = zr + qi, zi - qr
            st.setdefault("yr", []).append(yr.astype(bf16))
            st.setdefault("yi", []).append(yi.astype(bf16))

        def a_inverse():
            y = _mm(g_ref[...], jnp.concatenate(st["yr"] + st["yi"], axis=0))
            oa_buf[slot] = (q_buf[slot].astype(f32) * (y + st["skip"])).astype(bf16)

        h_scr[n_mem:n_row, :] = x_buf[slot].astype(f32)
        h = h_scr[...]
        row = jax.lax.broadcasted_iota(jnp.int32, (n_row, n_row), 0)
        col = jax.lax.broadcasted_iota(jnp.int32, (n_row, n_row), 1)
        mask = (row < n_mem) | (row >= col)
        qkv, og, acc = {}, {}, []

        def b_qkv(t):
            qkv[t] = [_mm(h, jnp.concatenate([w[t * hg + j] for j in range(hg)], axis=1))
                      for w in (wq, wk, wv)]

        def b_att(t):
            q, k, v = qkv.pop(t)
            outs = []
            for j in range(hg):
                sl = slice(j * dh, (j + 1) * dh)
                sc = jnp.where(mask, _mm_t(q[:, sl], k[:, sl]) * scale, -1000000000.0)
                e = jnp.exp(sc - jnp.max(sc, axis=-1, keepdims=True))
                den = jnp.sum(e, axis=-1, keepdims=True)
                outs.append(_mm(e, v[:, sl]) * (1.0 / den))
            og[t] = jnp.concatenate(outs, axis=1)

        def b_out(t):
            rows = slice(t * hg * dh, (t + 1) * hg * dh)
            y = _mm(og.pop(t), jnp.concatenate([wo[n, rows, :] for n in range(dm // 128)], axis=1))
            acc.append(acc.pop() + y if acc else y)

        for t in range(n_hg + 2):
            if t < n_hg:
                b_qkv(t)
            if t == 0:
                a_forward()
            if 0 <= t - 1 < n_hg:
                b_att(t - 1)
                a_mix((t - 1) * (_TB // n_hg), _TB // n_hg)
            if t == n_hg:
                a_inverse()
            if 0 <= t - 2 < n_hg:
                b_out(t - 2)

        h_scr[0:n_mem, :] = acc[0][0:n_mem]
        ob_buf[slot] = acc[0][n_mem:].astype(bf16)
        for cp in out_copies(s, slot):
            cp.start()
        return carry

    jax.lax.fori_loop(0, n_seg, step, 0)
    for s in (n_seg - 2, n_seg - 1):
        for cp in out_copies(s, s % 2):
            cp.wait()


@functools.partial(jax.jit, static_argnames=("B_seg_len",))
def pallas_concat_heads__ssm_conv_h3__memory_aug_recurrent_mem_tr__prompt_kernel(
    A_q: jax.Array,
    A_k: jax.Array,
    A_v: jax.Array,
    A_shift_k: jax.Array,
    A_ssm_k: jax.Array,
    A_ssm_D: jax.Array,
    B_x: jax.Array,
    B_mem0: jax.Array,
    B_Wq: jax.Array,
    B_Wk: jax.Array,
    B_Wv: jax.Array,
    B_Wo: jax.Array,
    B_seg_len: int,
):
    batch, s_len, da = A_q.shape
    dm, nh, dh = B_Wq.shape
    n_mem = B_mem0.shape[1]
    ks = A_shift_k.shape[1]
    seg = int(B_seg_len)
    n_seg = s_len // seg
    n_tb = s_len // _TB
    n_grp = n_seg // n_tb
    cg = da // n_grp
    assert batch == 1 and dh == 128 and n_grp * n_tb == n_seg and cg % 128 == 0
    assert B_x.shape == (1, s_len, dm) and ks <= 9

    f32, bf16 = jnp.float32, jnp.bfloat16
    fwd, inv = _dft_matrices()
    n_stage, dc = 3, 128
    hbm = pl.BlockSpec(memory_space=pl.ANY)
    vmem = pl.BlockSpec(memory_space=pltpu.VMEM)
    out = pl.pallas_call(
        functools.partial(_kernel, seg=seg, n_seg=n_seg, n_grp=n_grp, cg=cg),
        in_specs=[hbm, hbm, hbm, vmem, hbm, vmem, hbm, vmem, hbm, hbm, hbm, hbm, vmem, vmem],
        out_specs=hbm,
        out_shape=jax.ShapeDtypeStruct((s_len, da + dm), bf16),
        scratch_shapes=[
            pltpu.VMEM((nh, dm, dh), bf16),
            pltpu.VMEM((nh, dm, dh), bf16),
            pltpu.VMEM((nh, dm, dh), bf16),
            pltpu.VMEM((dm // 128, nh * dh, 128), bf16),
            pltpu.VMEM((n_stage, dc, nh, dh), bf16),
            pltpu.VMEM((n_mem + seg, dm), f32),
            pltpu.VMEM((n_seg + 1, 2 * _TB, cg), f32),
            pltpu.VMEM((n_seg + 1, 2 * _TB, cg), f32),
            pltpu.VMEM((n_grp, 2 * _TB, cg), f32),
            pltpu.VMEM((n_grp, 8 + _TB, cg), f32),
            pltpu.VMEM((n_grp, ks + 1, 8, cg), f32),
            pltpu.VMEM((2, _TB, cg), bf16),
            pltpu.VMEM((2, _TB, cg), bf16),
            pltpu.VMEM((2, _TB, cg), bf16),
            pltpu.VMEM((2, cg, _TB), bf16),
            pltpu.VMEM((2, seg, dm), bf16),
            pltpu.VMEM((2, _TB, cg), bf16),
            pltpu.VMEM((2, seg, dm), bf16),
            pltpu.SemaphoreType.DMA((n_stage,)),
            pltpu.SemaphoreType.DMA((dm // 128,)),
            pltpu.SemaphoreType.DMA((2, 5)),
            pltpu.SemaphoreType.DMA((2, 2)),
        ],
        compiler_params=pltpu.CompilerParams(vmem_limit_bytes=110 * 1024 * 1024),
    )(
        A_q.reshape(s_len, da), A_k.reshape(s_len, da), A_v.reshape(s_len, da),
        A_shift_k.T, A_ssm_k, A_ssm_D.reshape(1, da),
        B_x.reshape(s_len, dm), B_mem0.reshape(n_mem, dm),
        B_Wq, B_Wk, B_Wv, B_Wo.reshape(nh * dh, dm), fwd, inv,
    )
    return out.reshape(1, s_len, da + dm)
```

```python
import functools
import math

import jax
import jax.numpy as jnp
import numpy as np
import jax.experimental.pallas as pl
import jax.experimental.pallas.tpu as pltpu

_TB = 128
_HC = 8
_HG = 4
_PRE = 8


def _dft_matrices():
    n = np.arange(_TB)
    k = np.concatenate([np.arange(0, _TB, 2), np.arange(1, _TB, 2)])
    ang = np.pi * (((2 * k[:, None] + 1) * n[None, :]) % (4 * _TB)) / (2 * _TB)
    fwd = np.concatenate([np.cos(ang), -np.sin(ang)], axis=0)
    inv = fwd.T / _TB
    return fwd.astype(jnp.bfloat16), inv.astype(jnp.bfloat16)


def _mm(a, b):
    return jax.lax.dot_general(
        a, b, (((1,), (0,)), ((), ())), preferred_element_type=jnp.float32)


def _mm_t(a, b):
    return jax.lax.dot_general(
        a, b, (((1,), (1,)), ((), ())), preferred_element_type=jnp.float32)


def _kernel(q_hbm, k_hbm, v_hbm, sk_ref, hk_hbm, d_ref, x_hbm, mem_ref,
            wq_hbm, wk_hbm, wv_hbm, wo_hbm, f_ref, g_ref,
            out_hbm,
            wqkv, wo, stage, ostage, xsel_buf, xsel, pre, h_scr,
            xs, hs, zprev, kpad, skd, fg,
            q_buf, k_buf, v_buf, hk_buf, x_buf, o_buf,
            w_sem, xsel_sem, in_sem, out_sem):
    f32, bf16, u32 = jnp.float32, jnp.bfloat16, jnp.uint32
    dm, nh, dh = wq_hbm.shape
    n_seg, seg, _ = x_hbm.shape
    n_grp, _, cg = zprev.shape
    n_mem = mem_ref.shape[0]
    n_row = n_mem + seg
    tu = 2 * _TB
    n_p = n_seg // n_grp
    n_tb = 2 * n_p
    ks = sk_ref.shape[0]
    da = q_hbm.shape[1]
    zero_slot = n_grp * n_tb
    scale = dh ** (-0.5)

    def in_copies(p, slot):
        rows = pl.ds(pl.multiple_of(p * tu, tu), tu)
        pairs = ((x_hbm.at[pl.ds(p * n_grp, n_grp)], x_buf), (k_hbm.at[rows, :], k_buf),
                 (v_hbm.at[rows, :], v_buf), (q_hbm.at[rows, :], q_buf),
                 (hk_hbm.at[:, rows], hk_buf))
        return [pltpu.make_async_copy(src, dst.at[slot], in_sem.at[slot, i])
                for i, (src, dst) in enumerate(pairs)]

    def out_copy(p, slot):
        rows = pl.ds(pl.multiple_of(p * tu, tu), tu)
        return pltpu.make_async_copy(o_buf.at[slot], out_hbm.at[rows, :], out_sem.at[slot])

    n_chunk = nh // _HC
    oc_rows = ostage.shape[0]

    def w_copy(m, c):
        if m == 3:
            rows = pl.ds(pl.multiple_of(c * oc_rows, oc_rows), oc_rows)
            return pltpu.make_async_copy(wo_hbm.at[rows, :], ostage, w_sem.at[m])
        heads = pl.ds(pl.multiple_of(c * _HC, _HC), _HC)
        return pltpu.make_async_copy(
            (wq_hbm, wk_hbm, wv_hbm)[m].at[:, heads, :], stage.at[m], w_sem.at[m])

    def relayout(m, c, i, n):
        if m == 3:
            r = oc_rows // n
            r0 = pl.multiple_of(c * (oc_rows // 2) + i * (r // 2), r // 2)
            wo[pl.ds(r0, r // 2), :] = pltpu.bitcast(ostage[i * r:(i + 1) * r], u32)
            return
        u = dm // 16 // n
        for j in range(i * u, (i + 1) * u):
            wqkv[pl.ds(m * nh + c * _HC, _HC), j * 8:(j + 1) * 8, :] = pltpu.bitcast(
                jnp.swapaxes(stage[m, j * 16:(j + 1) * 16], 0, 1), u32)

    xsel_copy = pltpu.make_async_copy(
        x_hbm.at[:, pl.ds(seg - _PRE, _PRE), :], xsel_buf, xsel_sem)
    w_copy(0, 0).start()
    xsel_copy.start()
    w_copy(1, 0).start()
    w_copy(2, 0).start()

    h_scr[0:n_mem, :] = mem_ref[...].astype(f32)
    xs[zero_slot] = jnp.zeros(xs.shape[1:], f32)
    hs[zero_slot] = jnp.zeros(hs.shape[1:], f32)
    zprev[...] = jnp.zeros(zprev.shape, f32)
    kpad[:, 0:8, :] = jnp.zeros((n_grp, 8, cg), f32)
    fg[0:_TB] = pltpu.bitcast(f_ref[...], u32)
    fg[_TB:_TB + _TB // 2] = pltpu.bitcast(g_ref[:, 0:_TB], u32)
    fg[_TB + _TB // 2:] = pltpu.bitcast(g_ref[:, _TB:], u32)
    for g in range(n_grp):
        cols = slice(g * cg, (g + 1) * cg)
        for j in range(ks):
            skd[g, j] = jnp.broadcast_to(sk_ref[j:j + 1, cols].astype(f32), (8, cg))
        skd[g, ks] = jnp.broadcast_to(d_ref[:, cols].astype(f32), (8, cg))

    w_copy(0, 0).wait()
    w_copy(3, 0).start()
    relayout(0, 0, 0, 1)
    xsel_copy.wait()
    w_copy(0, 1).start()
    xsel[...] = xsel_buf[...].astype(f32).reshape(xsel.shape)

    def load_weights(c, carry):
        order = (1, 2, 3, 0)
        n_split = 4
        rows_per = xsel.shape[0] // (2 * n_split)
        more = c + 1 < n_chunk
        cur, nxt = jnp.minimum(c, n_chunk - 1), jnp.minimum(c + 1, n_chunk - 1)
        for i, m in enumerate(order):
            if m == 0:
                pl.when(more)(lambda: w_copy(0, nxt).wait())
            else:
                w_copy(m, c).wait()
            if i == 0:
                pl.when((c > 0) & more)(lambda: w_copy(0, nxt).start())

                @pl.when(c == n_chunk - 1)
                def _():
                    for cp in in_copies(0, 0):
                        cp.start()
            else:
                pl.when(more)(lambda: w_copy(order[i - 1], nxt).start())
            for j in range(_HC):
                head = (i // 2) * nh + c * _HC + j
                for u in range(n_split):
                    relayout(m, nxt if m == 0 else cur, j * n_split + u, _HC * n_split)
                    r0 = ((i % 2) * n_split + u) * rows_per
                    pre[head, r0:r0 + rows_per, :] = _mm(
                        xsel[r0:r0 + rows_per, :], pltpu.bitcast(wqkv[head], bf16))
        return carry

    jax.lax.fori_loop(0, n_chunk, load_weights, 0)

    n_hg = nh // _HG
    n_ot = dm // 256

    def step(g, p):
        slot = p & 1
        a = 2 * p
        cols = pl.ds(pl.multiple_of(g * cg, cg), cg)
        seg_rows = pl.ds(pl.multiple_of(g * seg, seg), seg)
        pre_rows = pl.ds(pl.multiple_of((p * n_grp + g) * _PRE, _PRE), _PRE)
        val = {}

        def a_forward():
            kf = k_buf[slot, :, cols].astype(f32)
            kpad[g, 8:8 + tu, :] = kf
            coef = lambda j: jnp.tile(skd[g, j], (tu // 8, 1))
            k_shift = kf * coef(0)
            for j in range(1, ks):
                k_shift = k_shift + kpad[g, 8 - j:8 - j + tu, :] * coef(j)
            kpad[g, 0:8, :] = kf[tu - 8:, :]
            kv = k_shift * v_buf[slot, :, cols].astype(f32)
            val["skip"] = kv * coef(ks)
            kvb = kv.astype(bf16)
            f = pltpu.bitcast(fg[0:_TB], bf16)
            for b in range(2):
                xs[g * n_tb + a + b] = _mm(f, kvb[b * _TB:(b + 1) * _TB])
            for b in range(2):
                hs[g * n_tb + a + b] = _mm_t(f, hk_buf[slot, cols, b * _TB:(b + 1) * _TB])

        lags_per_piece = 2

        def a_mix():
            ih = [jnp.where(j <= a + 1, g * n_tb + j, zero_slot) for j in range(n_tb)]
            ix = [jnp.where(j <= a + 1, g * n_tb + a + 1 - j, zero_slot) for j in range(n_tb)]
            for r0 in range(0, _TB, 8):
                re, im = pl.ds(r0, 8), pl.ds(_TB + r0, 8)
                z = [None] * 4

                def mac(o, x, h):
                    pr, pi = x[0] * h[0] - x[1] * h[1], x[0] * h[1] + x[1] * h[0]
                    z[o] = pr if z[o] is None else z[o] + pr
                    z[o + 1] = pi if z[o + 1] is None else z[o + 1] + pi

                h_old = None
                for j in range(n_tb):
                    x = (xs[ix[j], re, :], xs[ix[j], im, :])
                    h_new = (hs[ih[j], re, :], hs[ih[j], im, :])
                    mac(2, x, h_new)
                    if h_old is not None:
                        mac(0, x, h_old)
                    h_old = h_new
                    if (j + 1) % lags_per_piece == 0 and j + 1 < n_tb:
                        yield
                zr, zi = zprev[g, re, :], zprev[g, im, :]
                zprev[g, re, :] = z[2]
                zprev[g, im, :] = z[3]
                if r0 < _TB // 2:
                    y = (z[0] - zi, z[1] + zr, z[2] - z[1], z[3] + z[0])
                else:
                    y = (z[0] + zi, z[1] - zr, z[2] + z[1], z[3] - z[0])
                for i in range(4):
                    val.setdefault(("y", i), []).append(y[i])
                yield

        def a_inverse():
            gm = jnp.concatenate([pltpu.bitcast(fg[_TB:_TB + _TB // 2], bf16),
                                  pltpu.bitcast(fg[_TB + _TB // 2:], bf16)], axis=1)
            spec = jnp.concatenate(
                [jnp.concatenate(val["y", 2 * b] + val["y", 2 * b + 1], axis=0) for b in range(2)],
                axis=1)
            y = _mm(gm, spec.astype(bf16))
            y = jnp.concatenate([y[:, :cg], y[:, cg:]], axis=0)
            o_buf[slot, :, cols] = (
                q_buf[slot, :, cols].astype(f32) * (y + val["skip"])).astype(bf16)

        mixer = a_mix()
        pace_slot = jnp.where(p >= 0, zero_slot + 1, 0)
        n_piece = (_TB // 8) * (n_tb // lags_per_piece)
        n_tick = (n_hg - 2) * (3 * _HG + n_ot) - 8
        count = [0, 0]

        def tick(t):
            if t < 2:
                return
            count[0] += 1
            while count[1] < min(n_piece, count[0] * n_piece // n_tick):
                count[1] += 1
                xs[pace_slot, 0:8, :] = val["last"]
                hs[pace_slot, 0:8, :] = val["last"]
                next(mixer)

        h_scr[n_mem:n_row, :] = x_buf[slot, g].astype(f32)
        h = h_scr[...]
        row = jax.lax.broadcasted_iota(jnp.int32, (n_row, n_row), 0)
        col = jax.lax.broadcasted_iota(jnp.int32, (n_row, n_row), 1)
        mask = (row < n_mem) | (row >= col)

        def b_proj(m, t, j):
            tick(t)
            i = m * nh + t * _HG + j
            w = pltpu.bitcast(wqkv[i], bf16)
            if m < 2:
                r = jnp.concatenate([_mm(h[:n_row - _PRE], w), pre[i, pre_rows, :]], axis=0)
            else:
                r = _mm(h, w)
            val.setdefault((m, t), []).append(r)
            val["last"] = r[0:8]

        def b_scores(t):
            for q, k in zip(val.pop((0, t)), val.pop((1, t))):
                sc = jnp.where(mask, _mm_t(q, k.astype(bf16)), -1000000000.0 / scale)
                e = jnp.exp2((sc - jnp.max(sc, axis=-1, keepdims=True))
                             * (scale * math.log2(math.e)))
                den = jnp.sum(e, axis=-1, keepdims=True)
                val.setdefault(("e", t), []).append(
                    (e, pltpu.reciprocal(den, full_range=False)))

        def b_values(t):
            val["o", t] = jnp.concatenate(
                [_mm(e, v.astype(bf16)) * r
                 for (e, r), v in zip(val.pop(("e", t)), val.pop((2, t)))], axis=1)

        def b_out(t, ns):
            rows = slice(t * _HG * dh // 2, (t + 1) * _HG * dh // 2)
            for n in ns:
                tick(t + 2)
                y = _mm(val["o", t], pltpu.bitcast(wo[rows, n * 256:(n + 1) * 256], bf16))
                val["last"] = y[0:8, 128:256]
                val["acc", n] = val["acc", n] + y if t else y

        for t in range(n_hg):
            for j in range(_HG):
                b_proj(0, t, j)
                b_proj(2, t, j)
                b_proj(1, t, j)
                if t >= 2:
                    b_out(t - 2, [j])
                if t >= 1 and j == 0:
                    b_scores(t - 1)
                if t >= 1 and j == 2:
                    b_values(t - 1)
            if t == 0:
                a_forward()
        assert count[1] == n_piece
        b_out(n_hg - 2, [0])
        b_scores(n_hg - 1)
        b_out(n_hg - 2, range(1, n_ot))
        b_values(n_hg - 1)
        a_inverse()
        b_out(n_hg - 1, range(n_ot))

        out = jnp.concatenate([val["acc", n] for n in range(n_ot)], axis=1)
        h_scr[0:n_mem, :] = out[0:n_mem]
        o_buf[slot, seg_rows, da:] = out[n_mem:].astype(bf16)
        return p

    def block(p, carry):
        slot = p & 1
        for cp in in_copies(p, slot):
            cp.wait()
        pl.when(p >= 2)(lambda: out_copy(p - 2, slot).wait())

        @pl.when(p + 1 < n_p)
        def _():
            for cp in in_copies(p + 1, 1 - slot):
                cp.start()

        jax.lax.fori_loop(0, n_grp, step, p)
        out_copy(p, slot).start()
        return carry

    jax.lax.fori_loop(0, n_p, block, 0)
    for p in (n_p - 2, n_p - 1):
        out_copy(p, p % 2).wait()


@functools.partial(jax.jit, static_argnames=("B_seg_len",))
def pallas_concat_heads__ssm_conv_h3__memory_aug_recurrent_mem_tr__prompt_kernel(
    A_q: jax.Array,
    A_k: jax.Array,
    A_v: jax.Array,
    A_shift_k: jax.Array,
    A_ssm_k: jax.Array,
    A_ssm_D: jax.Array,
    B_x: jax.Array,
    B_mem0: jax.Array,
    B_Wq: jax.Array,
    B_Wk: jax.Array,
    B_Wv: jax.Array,
    B_Wo: jax.Array,
    B_seg_len: int,
):
    batch, s_len, da = A_q.shape
    dm, nh, dh = B_Wq.shape
    n_mem = B_mem0.shape[1]
    ks = A_shift_k.shape[1]
    seg = int(B_seg_len)
    n_seg = s_len // seg
    tu = 2 * _TB
    n_grp = tu // seg
    cg = da // n_grp
    assert batch == 1 and dh == 128 and cg == 128 and dm == 256 * _HG
    assert B_x.shape == (1, s_len, dm) and s_len % (2 * tu) == 0 and ks <= 9

    f32, bf16, u32 = jnp.float32, jnp.bfloat16, jnp.uint32
    fwd, inv = _dft_matrices()
    hbm = pl.BlockSpec(memory_space=pl.ANY)
    vmem = pl.BlockSpec(memory_space=pltpu.VMEM)
    out = pl.pallas_call(
        _kernel,
        in_specs=[hbm, hbm, hbm, vmem, hbm, vmem, hbm, vmem, hbm, hbm, hbm, hbm, vmem, vmem],
        out_specs=hbm,
        out_shape=jax.ShapeDtypeStruct((s_len, da + dm), bf16),
        scratch_shapes=[
            pltpu.VMEM((3 * nh, dm // 2, dh), u32),
            pltpu.VMEM((nh * dh // 2, dm), u32),
            pltpu.VMEM((3, dm, _HC, dh), bf16),
            pltpu.VMEM((_HC * dh, dm), bf16),
            pltpu.VMEM((n_seg, _PRE, dm), bf16),
            pltpu.VMEM((n_seg * _PRE, dm), f32),
            pltpu.VMEM((2 * nh, n_seg * _PRE, dh), f32),
            pltpu.VMEM((n_mem + seg, dm), f32),
            pltpu.VMEM((2 * n_seg + 2, 2 * _TB, cg), f32),
            pltpu.VMEM((2 * n_seg + 2, 2 * _TB, cg), f32),
            pltpu.VMEM((n_grp, 2 * _TB, cg), f32),
            pltpu.VMEM((n_grp, 8 + tu, cg), f32),
            pltpu.VMEM((n_grp, ks + 1, 8, cg), f32),
            pltpu.VMEM((2 * _TB, _TB), u32),
            pltpu.VMEM((2, tu, da), bf16),
            pltpu.VMEM((2, tu, da), bf16),
            pltpu.VMEM((2, tu, da), bf16),
            pltpu.VMEM((2, da, tu), bf16),
            pltpu.VMEM((2, n_grp, seg, dm), bf16),
            pltpu.VMEM((2, tu, da + dm), bf16),
            pltpu.SemaphoreType.DMA((4,)),
            pltpu.SemaphoreType.DMA(()),
            pltpu.SemaphoreType.DMA((2, 5)),
            pltpu.SemaphoreType.DMA((2,)),
        ],
        compiler_params=pltpu.CompilerParams(
            vmem_limit_bytes=120 * 1024 * 1024,
            flags={"XLA_TPU_EVENLY_DISTRIBUTE_CRITICAL_NODES": True}),
    )(
        A_q.reshape(s_len, da), A_k.reshape(s_len, da), A_v.reshape(s_len, da),
        A_shift_k.T, A_ssm_k, A_ssm_D.reshape(1, da),
        B_x.reshape(n_seg, seg, dm), B_mem0.reshape(n_mem, dm),
        B_Wq, B_Wk, B_Wv, B_Wo.reshape(nh * dh, dm), fwd, inv,
    )
    return out.reshape(1, s_len, da + dm)
```

```python
import functools
import math

import jax
import jax.numpy as jnp
import numpy as np
import jax.experimental.pallas as pl
import jax.experimental.pallas.tpu as pltpu

_TB = 128
_HC = 8
_HG = 4
_BOOT = 8
_PRE = 8


def _dft_matrices():
    n = np.arange(_TB)
    k = np.arange(0, _TB, 2)
    ang = np.pi * (((2 * k[:, None] + 1) * n[None, :]) % (4 * _TB)) / (2 * _TB)
    re, im, alt = np.cos(ang), -np.sin(ang), 1.0 - 2.0 * (n % 2)
    fwd = np.concatenate([re, re * alt, im, im * alt], axis=0)
    inv = np.concatenate([re, im], axis=0).T / _TB
    inv = np.concatenate([inv[0::2], inv[1::2]], axis=0)
    return np.concatenate([fwd, inv], axis=0).astype(jnp.bfloat16)


def _mm(a, b):
    return jax.lax.dot_general(
        a, b, (((1,), (0,)), ((), ())), preferred_element_type=jnp.float32)


def _mm_t(a, b):
    return jax.lax.dot_general(
        a, b, (((1,), (1,)), ((), ())), preferred_element_type=jnp.float32)


def _kernel(q_hbm, k_hbm, v_hbm, sk_hbm, hk_hbm, d_hbm, x_hbm, mem_hbm,
            wq_hbm, wk_hbm, wv_hbm, wo_hbm, dft_hbm,
            out_hbm,
            wqkv, wo, stage, ostage, xsel_buf, xsel, pre, h_scr,
            spec, zprev, kpad, skd, dft, ybuf,
            q_buf, k_buf, v_buf, hk_buf, x_buf, o_buf,
            sk_buf, d_buf, mem_buf, dft_buf,
            w_sem, boot_sem, small_sem, in_sem, out_sem):
    f32, bf16, u32 = jnp.float32, jnp.bfloat16, jnp.uint32
    dm, nh, dh = wq_hbm.shape
    n_seg, seg, _ = x_hbm.shape
    n_grp, _, cg = zprev.shape
    n_mem = mem_buf.shape[0]
    n_row = n_mem + seg
    tu = 2 * _TB
    n_p = n_seg // n_grp
    n_tb = 2 * n_p
    ks = sk_buf.shape[0]
    da = q_hbm.shape[1]
    zero_slot = n_grp * n_tb
    scale = dh ** (-0.5)
    x_re, x_im, h_re, h_im = (i * (_TB + 8) for i in range(4))

    def in_copies(p, slot):
        rows = pl.ds(pl.multiple_of(p * tu, tu), tu)
        pairs = ((x_hbm.at[pl.ds(p * n_grp, n_grp)], x_buf), (k_hbm.at[rows, :], k_buf),
                 (v_hbm.at[rows, :], v_buf), (q_hbm.at[rows, :], q_buf),
                 (hk_hbm.at[:, rows], hk_buf))
        return [pltpu.make_async_copy(src, dst.at[slot], in_sem.at[slot, i])
                for i, (src, dst) in enumerate(pairs)]

    def out_copy(p, slot):
        rows = pl.ds(pl.multiple_of(p * tu, tu), tu)
        return pltpu.make_async_copy(o_buf.at[slot], out_hbm.at[rows, :], out_sem.at[slot])

    n_chunk = nh // _HC
    oc_rows = ostage.shape[0]

    def w_copy(m, c):
        if m == 3:
            rows = pl.ds(pl.multiple_of(c * oc_rows, oc_rows), oc_rows)
            return pltpu.make_async_copy(wo_hbm.at[rows, :], ostage, w_sem.at[m])
        heads = pl.ds(pl.multiple_of(c * _HC, _HC), _HC)
        return pltpu.make_async_copy(
            (wq_hbm, wk_hbm, wv_hbm)[m].at[:, heads, :], stage.at[m], w_sem.at[m])

    def relayout(m, c, i, n):
        if m == 3:
            r = oc_rows // n
            r0 = pl.multiple_of(c * (oc_rows // 2) + i * (r // 2), r // 2)
            wo[pl.ds(r0, r // 2), :] = pltpu.bitcast(ostage[i * r:(i + 1) * r], u32)
            return
        u = dm // 16 // n
        for j in range(i * u, (i + 1) * u):
            wqkv[pl.ds(m * nh + c * _HC, _HC), j * 8:(j + 1) * 8, :] = pltpu.bitcast(
                jnp.swapaxes(stage[m, j * 16:(j + 1) * 16], 0, 1), u32)

    boot_rows, ahead = dm // _BOOT, _BOOT // 2

    def boot_copy(i):
        rows = pl.ds(pl.multiple_of(i * boot_rows, boot_rows), boot_rows)
        return pltpu.make_async_copy(
            wq_hbm.at[rows, 0:_HC, :], stage.at[0, rows], boot_sem.at[i])

    xsel_copy = pltpu.make_async_copy(
        x_hbm.at[:, pl.ds(seg - _PRE, _PRE), :], xsel_buf, boot_sem.at[_BOOT])
    small = [pltpu.make_async_copy(src, dst, small_sem.at[i]) for i, (src, dst) in enumerate(
        ((sk_hbm, sk_buf), (d_hbm, d_buf), (mem_hbm, mem_buf), (dft_hbm, dft_buf)))]
    for cp in small + [xsel_copy] + [boot_copy(i) for i in range(ahead - 1)]:
        cp.start()

    @pl.loop(0, oc_rows // 64)
    def _(i):
        ostage[pl.ds(pl.multiple_of(i * 64, 64), 64), :] = jnp.zeros((64, dm), bf16)

    spec[zero_slot] = jnp.zeros(spec.shape[1:], f32)

    @pl.loop(0, n_grp)
    def _(g):
        zprev[g] = jnp.zeros(zprev.shape[1:], f32)
        kpad[g, 0:8, :] = jnp.zeros((8, cg), f32)

    xsel_copy.wait()
    boot_copy(ahead - 1).start()

    @pl.loop(0, n_seg // 4)
    def _(i):
        rows = xsel_buf[pl.ds(i * 4, 4)].astype(f32).reshape(4 * _PRE, dm).astype(bf16)
        r0 = pl.multiple_of(i * 2 * _PRE, 2 * _PRE)
        xsel[pl.ds(r0, 2 * _PRE), :] = pltpu.bitcast(rows, u32)

    for cp in small:
        cp.wait()
    h_scr[0:n_mem, :] = mem_buf[...].astype(f32)
    dft[...] = pltpu.bitcast(dft_buf[...], u32)
    d_row = d_buf[...].astype(f32).reshape(1, da)
    for g in range(n_grp):
        cols = slice(g * cg, (g + 1) * cg)
        for j in range(ks):
            skd[g, j] = jnp.broadcast_to(sk_buf[j:j + 1, cols].astype(f32), (8, cg))
        skd[g, ks] = jnp.broadcast_to(d_row[:, cols], (8, cg))

    @pl.loop(0, _BOOT)
    def _(i):
        boot_copy(i).wait()
        pl.when(i + ahead < _BOOT)(lambda: boot_copy(i + ahead).start())
        pl.when(i == _BOOT - 2)(lambda: w_copy(1, 0).start())

        @pl.loop(0, boot_rows // 64)
        def _(j):
            r = i * boot_rows + j * 64
            wqkv[0:_HC, pl.ds(pl.multiple_of(r // 2, 32), 32), :] = pltpu.bitcast(
                jnp.swapaxes(stage[0, pl.ds(r, 64)], 0, 1), u32)

    def load_weights(c, carry):
        n_split = 4
        rows_per = n_seg * _PRE // (2 * n_split)
        more = c + 1 < n_chunk
        prv = jnp.maximum(c - 1, 0)
        cur = jnp.minimum(c, n_chunk - 1)
        nxt = jnp.minimum(c + 1, n_chunk - 1)
        for i, (m, chunk) in enumerate(((3, prv), (1, cur), (2, cur), (0, nxt))):
            if i == 0:
                pl.when(c > 0)(lambda: w_copy(3, prv).wait())
                w_copy(2, c).start()
            elif i == 1:
                w_copy(1, c).wait()
                pl.when(more)(lambda: w_copy(0, nxt).start())

                @pl.when(c == n_chunk - 1)
                def _():
                    for cp in in_copies(0, 0):
                        cp.start()
            elif i == 2:
                w_copy(2, c).wait()
                w_copy(3, c).start()
            else:
                pl.when(more)(lambda: w_copy(0, nxt).wait())
                pl.when(more)(lambda: w_copy(1, nxt).start())
            for j in range(_HC):
                head = (i // 2) * nh + c * _HC + j
                for u in range(n_split):
                    relayout(m, chunk, j * n_split + u, _HC * n_split)
                    r0 = ((i % 2) * n_split + u) * rows_per
                    pre[head, r0:r0 + rows_per, :] = _mm(
                        pltpu.bitcast(xsel[r0 // 2:(r0 + rows_per) // 2, :], bf16),
                        pltpu.bitcast(wqkv[head], bf16))
        return carry

    jax.lax.fori_loop(0, n_chunk, load_weights, 0)
    w_copy(3, n_chunk - 1).wait()

    @pl.loop(0, oc_rows // 64)
    def _(i):
        r0 = pl.multiple_of((n_chunk - 1) * (oc_rows // 2) + i * 32, 32)
        wo[pl.ds(r0, 32), :] = pltpu.bitcast(
            ostage[pl.ds(pl.multiple_of(i * 64, 64), 64), :], u32)

    n_hg = nh // _HG
    n_ot = dm // 256

    def step(g, p):
        slot = p & 1
        a = 2 * p
        cols = pl.ds(pl.multiple_of(g * cg, cg), cg)
        seg_rows = pl.ds(pl.multiple_of(g * seg, seg), seg)
        pre_rows = pl.ds(pl.multiple_of((p * n_grp + g) * _PRE, _PRE), _PRE)
        val = {}

        def a_filter():
            f = pltpu.bitcast(dft[0:_TB], bf16)
            for b in range(2):
                taps = hk_buf[slot, cols, b * _TB:(b + 1) * _TB]
                for o, part in ((h_re, f[:_TB]), (h_im, f[_TB:])):
                    spec[g * n_tb + a + b, o:o + _TB] = _mm_t(part, taps)

        def a_forward():
            kf = k_buf[slot, :, cols].astype(f32)
            kpad[g, 8:8 + tu, :] = kf
            coef = lambda j: jnp.tile(skd[g, j], (tu // 8, 1))
            k_shift = kf * coef(0)
            for j in range(1, ks):
                k_shift = k_shift + kpad[g, 8 - j:8 - j + tu, :] * coef(j)
            kpad[g, 0:8, :] = kf[tu - 8:, :]
            kv = k_shift * v_buf[slot, :, cols].astype(f32)
            val["skip"] = kv * coef(ks)
            kvb = kv.astype(bf16)
            f = pltpu.bitcast(dft[0:_TB], bf16)
            for b in range(2):
                for o, part in ((x_re, f[:_TB]), (x_im, f[_TB:])):
                    spec[g * n_tb + a + b, o:o + _TB] = _mm(part, kvb[b * _TB:(b + 1) * _TB])

        lags_per_piece = 2

        def a_mix():
            ih = [jnp.where(j <= a + 1, g * n_tb + j, zero_slot) for j in range(n_tb)]
            ix = [jnp.where(j <= a + 1, g * n_tb + a + 1 - j, zero_slot) for j in range(n_tb)]
            for r0 in [r + o for r in range(0, _TB // 2, 8) for o in (0, _TB // 2)]:
                at = lambda o: pl.ds(o + r0, 8)
                z = [None] * 4

                def mac(o, x, h):
                    pr, pi = x[0] * h[0] - x[1] * h[1], x[0] * h[1] + x[1] * h[0]
                    z[o] = pr if z[o] is None else z[o] + pr
                    z[o + 1] = pi if z[o + 1] is None else z[o + 1] + pi

                h_old = None
                for j in range(n_tb):
                    x = (spec[ix[j], at(x_re), :], spec[ix[j], at(x_im), :])
                    h_new = (spec[ih[j], at(h_re), :], spec[ih[j], at(h_im), :])
                    mac(2, x, h_new)
                    if h_old is not None:
                        mac(0, x, h_old)
                    h_old = h_new
                    if (j + 1) % lags_per_piece == 0 and j + 1 < n_tb:
                        yield
                zr, zi = zprev[g, at(0), :], zprev[g, at(_TB), :]
                zprev[g, at(0), :] = z[2]
                zprev[g, at(_TB), :] = z[3]
                y = (z[0] - zi, z[1] + zr, z[2] - z[1], z[3] + z[0])
                if r0 < _TB // 2:
                    y_lo = y
                else:
                    for i in range(4):
                        val.setdefault(("y", 0, i), []).append(y_lo[i] + y[i])
                        val.setdefault(("y", 1, i), []).append(y_lo[i] - y[i])
                yield

        def a_inverse():
            for par in range(2):
                r0 = _TB + par * _TB // 4
                inv = pltpu.bitcast(dft[r0:r0 + _TB // 4], bf16)
                for b in range(2):
                    y = jnp.concatenate(val["y", par, 2 * b] + val["y", par, 2 * b + 1], axis=0)
                    ybuf[pl.ds(b * _TB + par, _TB // 2, stride=2), :] = _mm(inv, y.astype(bf16))
            o_buf[slot, :, cols] = (
                q_buf[slot, :, cols].astype(f32) * (ybuf[0:tu] + val["skip"])).astype(bf16)

        mixer = a_mix()
        pace_slot = jnp.where(p >= 0, zero_slot + 1, 0)
        n_piece = (_TB // 8) * (n_tb // lags_per_piece)
        n_tick = (n_hg - 2) * (3 * _HG + n_ot) - 8
        count = [0, 0]

        def tick(t):
            if t < 2:
                return
            count[0] += 1
            while count[1] < min(n_piece, count[0] * n_piece // n_tick):
                count[1] += 1
                spec[pace_slot, 0:8, :] = val["last"]
                next(mixer)

        h_scr[n_mem:n_row, :] = x_buf[slot, g].astype(f32)
        h = h_scr[...]
        row = jax.lax.broadcasted_iota(jnp.int32, (n_row, n_row), 0)
        col = jax.lax.broadcasted_iota(jnp.int32, (n_row, n_row), 1)
        mask = (row < n_mem) | (row >= col)

        def b_proj(m, t, j):
            tick(t)
            i = m * nh + t * _HG + j
            w = pltpu.bitcast(wqkv[i], bf16)
            if m < 2:
                r = jnp.concatenate([_mm(h[:n_row - _PRE], w), pre[i, pre_rows, :]], axis=0)
            else:
                r = _mm(h, w)
            val.setdefault((m, t), []).append(r)
            val["last"] = r[0:8]

        def b_scores(t):
            for q, k in zip(val.pop((0, t)), val.pop((1, t))):
                sc = jnp.where(mask, _mm_t(q, k.astype(bf16)), -1000000000.0 / scale)
                e = jnp.exp2((sc - jnp.max(sc, axis=-1, keepdims=True))
                             * (scale * math.log2(math.e)))
                den = jnp.sum(e, axis=-1, keepdims=True)
                val.setdefault(("e", t), []).append(
                    (e, pltpu.reciprocal(den, full_range=False)))

        def b_values(t):
            val["o", t] = jnp.concatenate(
                [_mm(e, v.astype(bf16)) * r
                 for (e, r), v in zip(val.pop(("e", t)), val.pop((2, t)))], axis=1)

        def b_out(t, n):
            tick(t + 2)
            rows = slice(t * _HG * dh // 2, (t + 1) * _HG * dh // 2)
            y = _mm(val["o", t], pltpu.bitcast(wo[rows, n * 256:(n + 1) * 256], bf16))
            val["last"] = y[0:8, 128:256]
            val["acc", n] = val["acc", n] + y if t else y

        a_filter()
        outs = [(t, n) for t in range(n_hg) for n in range(n_ot)]
        for t in range(n_hg):
            for j in range(_HG):
                for m in range(3):
                    b_proj(m, t, j)
                if t >= 2 and len(outs) > 2 * n_ot + 2:
                    b_out(*outs.pop(0))
                if t >= 1 and j == 0:
                    b_scores(t - 1)
                if t >= 1 and j == _HG - 1:
                    b_values(t - 1)
                if (t, j) == (1, 0):
                    a_forward()
        assert count[1] == n_piece
        for i, tn in enumerate(outs):
            b_out(*tn)
            if i == 0:
                b_scores(n_hg - 1)
            if i == n_ot - 1:
                a_inverse()
                b_values(n_hg - 1)

        out = jnp.concatenate([val["acc", n] for n in range(n_ot)], axis=1)
        h_scr[0:n_mem, :] = out[0:n_mem]
        o_buf[slot, seg_rows, da:] = out[n_mem:].astype(bf16)
        return p

    def block(p, carry):
        slot = p & 1
        for cp in in_copies(p, slot):
            cp.wait()
        pl.when(p >= 2)(lambda: out_copy(p - 2, slot).wait())

        @pl.when(p + 1 < n_p)
        def _():
            for cp in in_copies(p + 1, 1 - slot):
                cp.start()

        jax.lax.fori_loop(0, n_grp, step, p, unroll=4)
        out_copy(p, slot).start()
        return carry

    jax.lax.fori_loop(0, n_p, block, 0)
    for p in (n_p - 2, n_p - 1):
        out_copy(p, p % 2).wait()


@functools.partial(jax.jit, static_argnames=("B_seg_len",))
def pallas_concat_heads__ssm_conv_h3__memory_aug_recurrent_mem_tr__prompt_kernel(
    A_q: jax.Array,
    A_k: jax.Array,
    A_v: jax.Array,
    A_shift_k: jax.Array,
    A_ssm_k: jax.Array,
    A_ssm_D: jax.Array,
    B_x: jax.Array,
    B_mem0: jax.Array,
    B_Wq: jax.Array,
    B_Wk: jax.Array,
    B_Wv: jax.Array,
    B_Wo: jax.Array,
    B_seg_len: int,
):
    batch, s_len, da = A_q.shape
    dm, nh, dh = B_Wq.shape
    n_mem = B_mem0.shape[1]
    ks = A_shift_k.shape[1]
    seg = int(B_seg_len)
    n_seg = s_len // seg
    tu = 2 * _TB
    n_grp = tu // seg
    cg = da // n_grp
    assert batch == 1 and dh == 128 and cg == 128 and dm == 256 * _HG
    assert B_x.shape == (1, s_len, dm) and s_len % (2 * tu) == 0 and ks <= 9

    f32, bf16, u32 = jnp.float32, jnp.bfloat16, jnp.uint32
    dft = _dft_matrices()
    hbm = pl.BlockSpec(memory_space=pl.ANY)
    out = pl.pallas_call(
        _kernel,
        in_specs=[hbm] * 13,
        out_specs=hbm,
        out_shape=jax.ShapeDtypeStruct((s_len, da + dm), bf16),
        scratch_shapes=[
            pltpu.VMEM((3 * nh, dm // 2, dh), u32),
            pltpu.VMEM((nh * dh // 2, dm), u32),
            pltpu.VMEM((3, dm, _HC, dh), bf16),
            pltpu.VMEM((_HC * dh, dm), bf16),
            pltpu.VMEM((n_seg, _PRE, dm), bf16),
            pltpu.VMEM((n_seg * _PRE // 2, dm), u32),
            pltpu.VMEM((2 * nh, n_seg * _PRE, dh), f32),
            pltpu.VMEM((n_mem + seg, dm), f32),
            pltpu.VMEM((2 * n_seg + 2, 4 * (_TB + 8), cg), f32),
            pltpu.VMEM((n_grp, 2 * _TB, cg), f32),
            pltpu.VMEM((n_grp, 8 + tu, cg), f32),
            pltpu.VMEM((n_grp, ks + 1, 8, cg), f32),
            pltpu.VMEM((dft.shape[0] // 2, _TB), u32),
            pltpu.VMEM((tu + 8, cg), f32),
            pltpu.VMEM((2, tu, da), bf16),
            pltpu.VMEM((2, tu, da), bf16),
            pltpu.VMEM((2, tu, da), bf16),
            pltpu.VMEM((2, da, tu), bf16),
            pltpu.VMEM((2, n_grp, seg, dm), bf16),
            pltpu.VMEM((2, tu, da + dm), bf16),
            pltpu.VMEM((ks, da), bf16),
            pltpu.VMEM((da,), bf16),
            pltpu.VMEM((n_mem, dm), bf16),
            pltpu.VMEM(dft.shape, bf16),
            pltpu.SemaphoreType.DMA((4,)),
            pltpu.SemaphoreType.DMA((_BOOT + 1,)),
            pltpu.SemaphoreType.DMA((4,)),
            pltpu.SemaphoreType.DMA((2, 5)),
            pltpu.SemaphoreType.DMA((2,)),
        ],
        compiler_params=pltpu.CompilerParams(
            vmem_limit_bytes=120 * 1024 * 1024,
            flags={"XLA_TPU_EVENLY_DISTRIBUTE_CRITICAL_NODES": True}),
    )(
        A_q.reshape(s_len, da), A_k.reshape(s_len, da), A_v.reshape(s_len, da),
        A_shift_k.T, A_ssm_k, A_ssm_D,
        B_x.reshape(n_seg, seg, dm), B_mem0.reshape(n_mem, dm),
        B_Wq, B_Wk, B_Wv, B_Wo.reshape(nh * dh, dm), dft,
    )
    return out.reshape(1, s_len, da + dm)
```

```python
import functools
import math

import jax
import jax.numpy as jnp
import numpy as np
import jax.experimental.pallas as pl
import jax.experimental.pallas.tpu as pltpu

_TB = 128
_HC = 8
_HG = 4
_BOOT = 8
_PRE = 8


def _dft_matrices():
    n = np.arange(_TB)
    k = np.arange(0, _TB, 2)
    ang = np.pi * (((2 * k[:, None] + 1) * n[None, :]) % (4 * _TB)) / (2 * _TB)
    re, im, alt = np.cos(ang), -np.sin(ang), 1.0 - 2.0 * (n % 2)
    fwd = np.concatenate([re, re * alt, im, im * alt], axis=0)
    inv = np.concatenate([re, im], axis=0).T / _TB
    split = np.concatenate([n[0::2], n[1::2]])
    return np.concatenate([fwd, fwd[:, split], inv[split]], axis=0).astype(jnp.bfloat16)


def _mm(a, b):
    return jax.lax.dot_general(
        a, b, (((1,), (0,)), ((), ())), preferred_element_type=jnp.float32)


def _mm_t(a, b):
    return jax.lax.dot_general(
        a, b, (((1,), (1,)), ((), ())), preferred_element_type=jnp.float32)


def _rows(words, par):
    bits = words & np.uint32(0xFFFF0000) if par else words << 16
    return pltpu.bitcast(bits, jnp.float32)


def _interleave(even, odd):
    even, odd = (pltpu.bitcast(x.astype(jnp.bfloat16).astype(jnp.float32), jnp.uint32)
                 for x in (even, odd))
    return pltpu.bitcast((even >> 16) | odd, jnp.bfloat16)


def _kernel(q_hbm, k_hbm, v_hbm, sk_hbm, hk_hbm, d_hbm, x_hbm, mem_hbm,
            wq_hbm, wk_hbm, wv_hbm, wo_hbm, dft_hbm,
            out_hbm,
            wqkv, wo, stage, ostage, xsel_buf, xsel, pre, h_scr,
            spec, zprev, ktail, skd, dft,
            q_buf, k_buf, v_buf, hk_buf, x_buf, o_buf,
            sk_buf, d_buf, mem_buf, dft_buf,
            w_sem, boot_sem, small_sem, in_sem, out_sem):
    f32, bf16, u32 = jnp.float32, jnp.bfloat16, jnp.uint32
    dm, nh, dh = wq_hbm.shape
    n_seg, seg, _ = x_hbm.shape
    n_grp, _, cg = zprev.shape
    n_mem = mem_buf.shape[0]
    n_row = n_mem + seg
    tu = 2 * _TB
    n_p = n_seg // n_grp
    n_tb = 2 * n_p
    ks = sk_buf.shape[0]
    da = q_hbm.shape[1]
    zero_slot = n_grp * n_tb
    scale = dh ** (-0.5)
    x_re, x_im, h_re, h_im = (i * (_TB + 8) for i in range(4))

    def in_copies(p, slot):
        rows = pl.ds(pl.multiple_of(p * tu, tu), tu)
        pairs = ((x_hbm.at[pl.ds(p * n_grp, n_grp)], x_buf), (k_hbm.at[rows, :], k_buf),
                 (v_hbm.at[rows, :], v_buf), (q_hbm.at[rows, :], q_buf),
                 (hk_hbm.at[:, rows], hk_buf))
        return [pltpu.make_async_copy(src, dst.at[slot], in_sem.at[slot, i])
                for i, (src, dst) in enumerate(pairs)]

    def out_copy(p, slot):
        rows = pl.ds(pl.multiple_of(p * tu, tu), tu)
        return pltpu.make_async_copy(o_buf.at[slot], out_hbm.at[rows, :], out_sem.at[slot])

    n_chunk = nh // _HC
    oc_rows = ostage.shape[0]

    def w_copy(m, c):
        if m == 3:
            rows = pl.ds(pl.multiple_of(c * oc_rows, oc_rows), oc_rows)
            return pltpu.make_async_copy(wo_hbm.at[rows, :], ostage, w_sem.at[m])
        heads = pl.ds(pl.multiple_of(c * _HC, _HC), _HC)
        return pltpu.make_async_copy(
            (wq_hbm, wk_hbm, wv_hbm)[m].at[:, heads, :], stage.at[m], w_sem.at[m])

    def relayout(m, c, i, n):
        if m == 3:
            r = oc_rows // n
            r0 = pl.multiple_of(c * (oc_rows // 2) + i * (r // 2), r // 2)
            wo[pl.ds(r0, r // 2), :] = pltpu.bitcast(ostage[i * r:(i + 1) * r], u32)
            return
        u = dm // 16 // n
        for j in range(i * u, (i + 1) * u):
            wqkv[pl.ds(m * nh + c * _HC, _HC), j * 8:(j + 1) * 8, :] = pltpu.bitcast(
                jnp.swapaxes(stage[m, j * 16:(j + 1) * 16], 0, 1), u32)

    boot_rows, ahead = dm // _BOOT, _BOOT // 2

    def boot_copy(i):
        rows = pl.ds(pl.multiple_of(i * boot_rows, boot_rows), boot_rows)
        return pltpu.make_async_copy(
            wq_hbm.at[rows, 0:_HC, :], stage.at[0, rows], boot_sem.at[i])

    xsel_copy = pltpu.make_async_copy(
        x_hbm.at[:, pl.ds(seg - _PRE, _PRE), :], xsel_buf, boot_sem.at[_BOOT])
    small = [pltpu.make_async_copy(src, dst, small_sem.at[i]) for i, (src, dst) in enumerate(
        ((sk_hbm, sk_buf), (d_hbm, d_buf), (mem_hbm, mem_buf), (dft_hbm, dft_buf)))]
    for cp in small + [xsel_copy] + [boot_copy(i) for i in range(ahead - 1)]:
        cp.start()

    @pl.loop(0, oc_rows // 64)
    def _(i):
        ostage[pl.ds(pl.multiple_of(i * 64, 64), 64), :] = jnp.zeros((64, dm), bf16)

    spec[zero_slot] = jnp.zeros(spec.shape[1:], f32)

    @pl.loop(0, n_grp)
    def _(g):
        zprev[g] = jnp.zeros(zprev.shape[1:], f32)
        ktail[g] = jnp.zeros((8, cg), u32)

    xsel_copy.wait()
    boot_copy(ahead - 1).start()

    @pl.loop(0, n_seg // 4)
    def _(i):
        rows = xsel_buf[pl.ds(i * 4, 4)].astype(f32).reshape(4 * _PRE, dm).astype(bf16)
        r0 = pl.multiple_of(i * 2 * _PRE, 2 * _PRE)
        xsel[pl.ds(r0, 2 * _PRE), :] = pltpu.bitcast(rows, u32)

    for cp in small:
        cp.wait()
    h_scr[0:n_mem, :] = mem_buf[...].astype(f32)
    dft[...] = pltpu.bitcast(dft_buf[...], u32)
    d_row = d_buf[...].astype(f32).reshape(1, da)
    for g in range(n_grp):
        cols = slice(g * cg, (g + 1) * cg)
        for j in range(ks):
            skd[g, j] = jnp.broadcast_to(sk_buf[j:j + 1, cols].astype(f32), (8, cg))
        skd[g, ks] = jnp.broadcast_to(d_row[:, cols], (8, cg))

    @pl.loop(0, _BOOT)
    def _(i):
        boot_copy(i).wait()
        pl.when(i + ahead < _BOOT)(lambda: boot_copy(i + ahead).start())
        pl.when(i == _BOOT - 2)(lambda: w_copy(1, 0).start())

        @pl.loop(0, boot_rows // 64)
        def _(j):
            r = i * boot_rows + j * 64
            wqkv[0:_HC, pl.ds(pl.multiple_of(r // 2, 32), 32), :] = pltpu.bitcast(
                jnp.swapaxes(stage[0, pl.ds(r, 64)], 0, 1), u32)

    def load_weights(c, carry):
        n_split = 4
        rows_per = n_seg * _PRE // (2 * n_split)
        more = c + 1 < n_chunk
        prv = jnp.maximum(c - 1, 0)
        cur = jnp.minimum(c, n_chunk - 1)
        nxt = jnp.minimum(c + 1, n_chunk - 1)
        for i, (m, chunk) in enumerate(((3, prv), (1, cur), (2, cur), (0, nxt))):
            if i == 0:
                pl.when(c > 0)(lambda: w_copy(3, prv).wait())
                w_copy(2, c).start()
            elif i == 1:
                w_copy(1, c).wait()
                pl.when(more)(lambda: w_copy(0, nxt).start())

                @pl.when(c == n_chunk - 1)
                def _():
                    for cp in in_copies(0, 0):
                        cp.start()
            elif i == 2:
                w_copy(2, c).wait()
                w_copy(3, c).start()
            else:
                pl.when(more)(lambda: w_copy(0, nxt).wait())
                pl.when(more)(lambda: w_copy(1, nxt).start())
            for j in range(_HC):
                head = (i // 2) * nh + c * _HC + j
                for u in range(n_split):
                    relayout(m, chunk, j * n_split + u, _HC * n_split)
                    r0 = ((i % 2) * n_split + u) * rows_per
                    pre[head, r0:r0 + rows_per, :] = _mm(
                        pltpu.bitcast(xsel[r0 // 2:(r0 + rows_per) // 2, :], bf16),
                        pltpu.bitcast(wqkv[head], bf16))
        return carry

    jax.lax.fori_loop(0, n_chunk, load_weights, 0)
    w_copy(3, n_chunk - 1).wait()

    @pl.loop(0, oc_rows // 64)
    def _(i):
        r0 = pl.multiple_of((n_chunk - 1) * (oc_rows // 2) + i * 32, 32)
        wo[pl.ds(r0, 32), :] = pltpu.bitcast(
            ostage[pl.ds(pl.multiple_of(i * 64, 64), 64), :], u32)

    n_hg = nh // _HG
    n_ot = dm // 256

    def step(g, p):
        slot = p & 1
        a = 2 * p
        cols = pl.ds(pl.multiple_of(g * cg, cg), cg)
        seg_rows = pl.ds(pl.multiple_of(g * seg, seg), seg)
        pre_rows = pl.ds(pl.multiple_of((p * n_grp + g) * _PRE, _PRE), _PRE)
        val = {}

        def a_filter():
            f = pltpu.bitcast(dft[0:_TB], bf16)
            for b in range(2):
                taps = hk_buf[slot, cols, b * _TB:(b + 1) * _TB]
                for o, part in ((h_re, f[:_TB]), (h_im, f[_TB:])):
                    spec[g * n_tb + a + b, o:o + _TB] = _mm_t(part, taps)

        def a_forward(b):
            hw = _TB // 2
            kw = pltpu.bitcast(k_buf[slot, b * _TB:(b + 1) * _TB, cols], u32)
            vw = pltpu.bitcast(v_buf[slot, b * _TB:(b + 1) * _TB, cols], u32)
            ext = jnp.concatenate([ktail[g], kw], axis=0)
            ktail[g] = kw[hw - 8:]
            past = [kw] + [ext[8 - i:8 - i + hw] for i in range(1, ks // 2 + 1)]
            coef = lambda j: jnp.tile(skd[g, j], (hw // 8, 1))
            kv = []
            for par in range(2):
                terms = [_rows(past[(j - par + 1) // 2], (par - j) % 2) * coef(j)
                         for j in range(ks)]
                kv.append(functools.reduce(jnp.add, terms) * _rows(vw, par))
                val["skip", par, b] = kv[par] * coef(ks)
            f = pltpu.bitcast(dft[_TB:2 * _TB], bf16)
            blk = jnp.concatenate(kv, axis=0).astype(bf16)
            for i, o in enumerate((x_re, x_re + hw, x_im, x_im + hw)):
                spec[g * n_tb + a + b, o:o + hw] = _mm(f[i * hw:(i + 1) * hw], blk)

        lags_per_piece = 2

        def a_mix():
            ih = [jnp.where(j <= a + 1, g * n_tb + j, zero_slot) for j in range(n_tb)]
            ix = [jnp.where(j <= a + 1, g * n_tb + a + 1 - j, zero_slot) for j in range(n_tb)]
            for r0 in [r + o for r in range(0, _TB // 2, 8) for o in (0, _TB // 2)]:
                at = lambda o: pl.ds(o + r0, 8)
                z = [None] * 4

                def mac(o, x, h):
                    pr, pi = x[0] * h[0] - x[1] * h[1], x[0] * h[1] + x[1] * h[0]
                    z[o] = pr if z[o] is None else z[o] + pr
                    z[o + 1] = pi if z[o + 1] is None else z[o + 1] + pi

                h_old = None
                for j in range(n_tb):
                    x = (spec[ix[j], at(x_re), :], spec[ix[j], at(x_im), :])
                    h_new = (spec[ih[j], at(h_re), :], spec[ih[j], at(h_im), :])
                    mac(2, x, h_new)
                    if h_old is not None:
                        mac(0, x, h_old)
                    h_old = h_new
                    if (j + 1) % lags_per_piece == 0 and j + 1 < n_tb:
                        yield
                zr, zi = zprev[g, at(0), :], zprev[g, at(_TB), :]
                zprev[g, at(0), :] = z[2]
                zprev[g, at(_TB), :] = z[3]
                y = (z[0] - zi, z[1] + zr, z[2] - z[1], z[3] + z[0])
                if r0 < _TB // 2:
                    y_lo = y
                else:
                    for i in range(4):
                        val.setdefault(("y", 0, i), []).append(y_lo[i] + y[i])
                        val.setdefault(("y", 1, i), []).append(y_lo[i] - y[i])
                yield

        def a_inverse():
            qw = pltpu.bitcast(q_buf[slot, :, cols], u32)
            res = []
            for par in range(2):
                r0 = 2 * _TB + par * _TB // 4
                inv = pltpu.bitcast(dft[r0:r0 + _TB // 4], bf16)
                y = [_mm(inv, jnp.concatenate(
                    val["y", par, 2 * b] + val["y", par, 2 * b + 1], axis=0).astype(bf16))
                     + val["skip", par, b] for b in range(2)]
                res.append(_rows(qw, par) * jnp.concatenate(y, axis=0))
            o_buf[slot, :, cols] = _interleave(*res)

        mixer = a_mix()
        pace_slot = jnp.where(p >= 0, zero_slot + 1, 0)
        n_piece = (_TB // 8) * (n_tb // lags_per_piece)
        n_tick = (n_hg - 1) * 3 * _HG + (n_hg - 2) * n_ot - 5
        count = [0, 0]

        def tick():
            count[0] += 1
            while count[1] < min(n_piece, count[0] * n_piece // n_tick):
                count[1] += 1
                spec[pace_slot, 0:8, :] = val["last"]
                next(mixer)

        h_scr[n_mem:n_row, :] = x_buf[slot, g].astype(f32)
        h = h_scr[...]
        row = jax.lax.broadcasted_iota(jnp.int32, (n_row, n_row), 0)
        col = jax.lax.broadcasted_iota(jnp.int32, (n_row, n_row), 1)
        mask = (row < n_mem) | (row >= col)

        def b_proj(m, t, j):
            if t >= 1:
                tick()
            i = m * nh + t * _HG + j
            w = pltpu.bitcast(wqkv[i], bf16)
            if m < 2:
                r = jnp.concatenate([_mm(h[:n_row - _PRE], w), pre[i, pre_rows, :]], axis=0)
            else:
                r = _mm(h, w)
            val.setdefault((m, t), []).append(r)
            val["last"] = r[0:8]

        def b_scores(t):
            for q, k in zip(val.pop((0, t)), val.pop((1, t))):
                sc = jnp.where(mask, _mm_t(q, k.astype(bf16)), -1000000000.0 / scale)
                e = jnp.exp2((sc - jnp.max(sc, axis=-1, keepdims=True))
                             * (scale * math.log2(math.e)))
                den = jnp.sum(e, axis=-1, keepdims=True)
                val.setdefault(("e", t), []).append(
                    (e, pltpu.reciprocal(den, full_range=False)))

        def b_values(t):
            val["o", t] = jnp.concatenate(
                [_mm(e, v.astype(bf16)) * r
                 for (e, r), v in zip(val.pop(("e", t)), val.pop((2, t)))], axis=1)

        def b_out(t, n):
            tick()
            rows = slice(t * _HG * dh // 2, (t + 1) * _HG * dh // 2)
            y = _mm(val["o", t], pltpu.bitcast(wo[rows, n * 256:(n + 1) * 256], bf16))
            val["last"] = y[0:8, 128:256]
            val["acc", n] = val["acc", n] + y if t else y

        a_filter()
        outs = [(t, n) for t in range(n_hg) for n in range(n_ot)]
        for t in range(n_hg):
            for j in range(_HG):
                for m in range(3):
                    b_proj(m, t, j)
                if t >= 2 and len(outs) > 2 * n_ot + 2:
                    b_out(*outs.pop(0))
                if t >= 1 and j == 0:
                    b_scores(t - 1)
                if t >= 1 and j == _HG - 1:
                    b_values(t - 1)
                if t == 0 and j % 2 == 1:
                    a_forward(j // 2)
        assert count[1] == n_piece
        for i, tn in enumerate(outs):
            b_out(*tn)
            if i == 0:
                b_scores(n_hg - 1)
            if i == n_ot - 1:
                b_values(n_hg - 1)
            if i == n_ot + 1:
                a_inverse()

        out = jnp.concatenate([val["acc", n] for n in range(n_ot)], axis=1)
        h_scr[0:n_mem, :] = out[0:n_mem]
        o_buf[slot, seg_rows, da:] = out[n_mem:].astype(bf16)
        return p

    def block(p, carry):
        slot = p & 1
        for cp in in_copies(p, slot):
            cp.wait()
        pl.when(p >= 2)(lambda: out_copy(p - 2, slot).wait())

        @pl.when(p + 1 < n_p)
        def _():
            for cp in in_copies(p + 1, 1 - slot):
                cp.start()

        jax.lax.fori_loop(0, n_grp, step, p, unroll=4)
        out_copy(p, slot).start()
        return carry

    jax.lax.fori_loop(0, n_p, block, 0)
    for p in (n_p - 2, n_p - 1):
        out_copy(p, p % 2).wait()


@functools.partial(jax.jit, static_argnames=("B_seg_len",))
def pallas_concat_heads__ssm_conv_h3__memory_aug_recurrent_mem_tr__prompt_kernel(
    A_q: jax.Array,
    A_k: jax.Array,
    A_v: jax.Array,
    A_shift_k: jax.Array,
    A_ssm_k: jax.Array,
    A_ssm_D: jax.Array,
    B_x: jax.Array,
    B_mem0: jax.Array,
    B_Wq: jax.Array,
    B_Wk: jax.Array,
    B_Wv: jax.Array,
    B_Wo: jax.Array,
    B_seg_len: int,
):
    batch, s_len, da = A_q.shape
    dm, nh, dh = B_Wq.shape
    n_mem = B_mem0.shape[1]
    ks = A_shift_k.shape[1]
    seg = int(B_seg_len)
    n_seg = s_len // seg
    tu = 2 * _TB
    n_grp = tu // seg
    cg = da // n_grp
    assert batch == 1 and dh == 128 and cg == 128 and dm == 256 * _HG
    assert B_x.shape == (1, s_len, dm) and s_len % (2 * tu) == 0 and ks <= 9

    f32, bf16, u32 = jnp.float32, jnp.bfloat16, jnp.uint32
    dft = _dft_matrices()
    hbm = pl.BlockSpec(memory_space=pl.ANY)
    out = pl.pallas_call(
        _kernel,
        in_specs=[hbm] * 13,
        out_specs=hbm,
        out_shape=jax.ShapeDtypeStruct((s_len, da + dm), bf16),
        scratch_shapes=[
            pltpu.VMEM((3 * nh, dm // 2, dh), u32),
            pltpu.VMEM((nh * dh // 2, dm), u32),
            pltpu.VMEM((3, dm, _HC, dh), bf16),
            pltpu.VMEM((_HC * dh, dm), bf16),
            pltpu.VMEM((n_seg, _PRE, dm), bf16),
            pltpu.VMEM((n_seg * _PRE // 2, dm), u32),
            pltpu.VMEM((2 * nh, n_seg * _PRE, dh), f32),
            pltpu.VMEM((n_mem + seg, dm), f32),
            pltpu.VMEM((2 * n_seg + 2, 4 * (_TB + 8), cg), f32),
            pltpu.VMEM((n_grp, 2 * _TB, cg), f32),
            pltpu.VMEM((n_grp, 8, cg), u32),
            pltpu.VMEM((n_grp, ks + 1, 8, cg), f32),
            pltpu.VMEM((dft.shape[0] // 2, _TB), u32),
            pltpu.VMEM((2, tu, da), bf16),
            pltpu.VMEM((2, tu, da), bf16),
            pltpu.VMEM((2, tu, da), bf16),
            pltpu.VMEM((2, da, tu), bf16),
            pltpu.VMEM((2, n_grp, seg, dm), bf16),
            pltpu.VMEM((2, tu, da + dm), bf16),
            pltpu.VMEM((ks, da), bf16),
            pltpu.VMEM((da,), bf16),
            pltpu.VMEM((n_mem, dm), bf16),
            pltpu.VMEM(dft.shape, bf16),
            pltpu.SemaphoreType.DMA((4,)),
            pltpu.SemaphoreType.DMA((_BOOT + 1,)),
            pltpu.SemaphoreType.DMA((4,)),
            pltpu.SemaphoreType.DMA((2, 5)),
            pltpu.SemaphoreType.DMA((2,)),
        ],
        compiler_params=pltpu.CompilerParams(
            vmem_limit_bytes=120 * 1024 * 1024,
            flags={"XLA_TPU_EVENLY_DISTRIBUTE_CRITICAL_NODES": True}),
    )(
        A_q.reshape(s_len, da), A_k.reshape(s_len, da), A_v.reshape(s_len, da),
        A_shift_k.T, A_ssm_k, A_ssm_D,
        B_x.reshape(n_seg, seg, dm), B_mem0.reshape(n_mem, dm),
        B_Wq, B_Wk, B_Wv, B_Wo.reshape(nh * dh, dm), dft,
    )
    return out.reshape(1, s_len, da + dm)
```
